```python
import jax
import jax.numpy as jnp

def _softmax(x, axis=-1):
    return jax.nn.softmax(x, axis=axis)
def _gelu(x):
    return jax.nn.gelu(x, approximate=True)
def _silu(x):
    return jax.nn.silu(x)
def _sigmoid(x):
    return jax.nn.sigmoid(x)
def _layernorm(x, axis=-1, eps=1e-5):
    m = jnp.mean(x, axis=axis, keepdims=True)
    v = jnp.var(x, axis=axis, keepdims=True)
    return (x - m) / jnp.sqrt(v + eps)
def _scatter_add(tgt, idx, src, axis=0):
    return tgt.at[idx].add(src)
def _segment_sum(src, seg, n):
    return jax.ops.segment_sum(src, seg, n)
class _Rng:
    def __init__(self, key):
        self._k = key
    def _next(self):
        self._k, sub = jax.random.split(self._k)
        return sub
    def normal(self, shape):
        return jax.random.normal(self._next(), shape, dtype=jnp.bfloat16)
    def randint(self, lo, hi, shape):
        return jax.random.randint(self._next(), shape, lo, hi, dtype=jnp.int32)
    def uniform(self, shape, lo=0.0, hi=1.0):
        return jax.random.uniform(self._next(), shape, jnp.bfloat16, lo, hi)
    def permutation(self, n):
        return jax.random.permutation(self._next(), n)


kernel_name = 'sequential_preLN__sliding_block_cached__glu_gated_swiglu__decode'

def setup_inputs():
    _rng = _Rng(jax.random.key(int.from_bytes(__import__("os").urandom(4), "little")))
    _w = (lambda a: (lambda t: t.astype(jnp.bfloat16) if jnp.issubdtype(t.dtype, jnp.floating) else t)(jnp.asarray(a)))
    def _A_setup():
        B, Sq, D = 1, 1, 640
        Hq, Hkv, Sk, Dh = 32, 32, 32768, 192
        assert Hq % Hkv == 0, (Hq, Hkv)
        return {
            "x": _w((lambda *s: _rng.normal(s) * 0.05)(B, Sq, D)),
            "k_cache": _w((lambda *s: _rng.normal(s) * 0.05)(B, Hkv, Sk, Dh)),
            "v_cache": _w((lambda *s: _rng.normal(s) * 0.05)(B, Hkv, Sk, Dh)),
            "wq": _w((lambda *s: _rng.normal(s) * 0.05)(D, Hq * Dh) * (D ** -0.5)),
            "wo": _w((lambda *s: _rng.normal(s) * 0.05)(Hq * Dh, D) * ((Hq * Dh) ** -0.5)),
        }
    _A_in = _A_setup()

    def _B_setup():
        B, S, D, F = 1, 1, 640, 1536
        return {
            "x": _w((lambda *s: _rng.normal(s) * 0.05)(B, S, D)),
            "w1": _w((lambda *s: _rng.normal(s) * 0.05)(D, F) * (2.0 / D) ** 0.5),
            "w3": _w((lambda *s: _rng.normal(s) * 0.05)(D, F) * (2.0 / D) ** 0.5),
            "w2": _w((lambda *s: _rng.normal(s) * 0.05)(F, D) * (2.0 / F) ** 0.5),
        }
    _B_in = _B_setup()

    return {
        "A_x": _A_in["x"],
        "A_k_cache": _A_in["k_cache"],
        "A_v_cache": _A_in["v_cache"],
        "A_wq": _A_in["wq"],
        "A_wo": _A_in["wo"],
        "B_x": _B_in["x"],
        "B_w1": _B_in["w1"],
        "B_w3": _B_in["w3"],
        "B_w2": _B_in["w2"],
    }

def reference(A_x, A_k_cache, A_v_cache, A_wq, A_wo, B_x, B_w1, B_w3, B_w2):
    def _A_ref(x, k_cache, v_cache, wq, wo):
        B, Sq, D = x.shape
        Hq, Dh = 32, 192
        Hkv, Sk = k_cache.shape[1], k_cache.shape[2]
        W = min(4096, max(256, Sk // 4))
        rep = Hq // Hkv
        q = (lambda x, *d: x.transpose(*d))((x @ wq).reshape(B, Sq, Hq, Dh), 0, 2, 1, 3)
        k = jnp.repeat(k_cache[:, :, Sk - W:, :], rep, axis=1)
        v = jnp.repeat(v_cache[:, :, Sk - W:, :], rep, axis=1)
        scores = jnp.einsum("bhqd,bhkd->bhqk", q, k) * (Dh ** -0.5)
        p = _softmax(scores, axis=-1)
        o = jnp.einsum("bhqk,bhkd->bhqd", p, v)
        return (lambda x, *d: x.transpose(*d))(o, 0, 2, 1, 3).reshape(B, Sq, Hq * Dh) @ wo

    def _B_ref(x, w1, w3, w2):
        gate = jnp.einsum("bsd,df->bsf", x, w1)
        up = jnp.einsum("bsd,df->bsf", x, w3)
        h = _silu(gate) * up
        out = jnp.einsum("bsf,fd->bsd", h, w2)
        return out

    x = A_x
    h = x + _A_ref(_layernorm(x, axis=-1), A_k_cache, A_v_cache, A_wq, A_wo)
    h2 = h + _B_ref(_layernorm(h, axis=-1), B_w1, B_w3, B_w2)
    return h2
```

```python
import functools
import jax
import jax.numpy as jnp
from jax import lax
from jax.experimental import pallas as pl
from jax.experimental.pallas import tpu as pltpu

D = 640
H = 32
DH = 192
SK = 32768
W = 4096
F = 1536
PAIR = 2 * DH
NPAIR = H // 2
EPS = 1e-5


def _layernorm(x):
    m = jnp.mean(x, axis=-1, keepdims=True)
    c = x - m
    v = jnp.mean(c * c, axis=-1, keepdims=True)
    return c * lax.rsqrt(v + EPS)


def make(nslots=3, nq=1, compute=True):
    def kernel(x_hbm, k_hbm, v_hbm, wq_hbm, wo_hbm, w1_hbm, w3_hbm, w2_hbm, o_ref,
               x_buf, wq_buf, wo_buf, w1_buf, w3_buf, w2_buf, kbuf, vbuf, q_scr, a_scr,
               wsem, kvsem):
        def x_copy():
            return pltpu.make_async_copy(x_hbm, x_buf, wsem.at[0])
        def wq_copy():
            return pltpu.make_async_copy(wq_hbm, wq_buf, wsem.at[1])
        def wo_copy():
            return pltpu.make_async_copy(wo_hbm, wo_buf, wsem.at[2])
        def w1_copy():
            return pltpu.make_async_copy(w1_hbm, w1_buf, wsem.at[3])
        def w3_copy():
            return pltpu.make_async_copy(w3_hbm, w3_buf, wsem.at[4])
        def w2_copy():
            return pltpu.make_async_copy(w2_hbm, w2_buf, wsem.at[5])
        def k_copy(i, slot):
            return pltpu.make_async_copy(
                k_hbm.at[pl.ds(i * PAIR, PAIR), pl.ds(SK - W, W)], kbuf.at[slot], kvsem.at[0, slot])
        def v_copy(i, slot):
            return pltpu.make_async_copy(
                v_hbm.at[pl.ds(i * PAIR, PAIR), pl.ds(SK - W, W)], vbuf.at[slot], kvsem.at[1, slot])

        x_copy().start()
        wq_copy().start()
        for i in range(nslots):
            k_copy(i, i).start()
            v_copy(i, i).start()

        x_copy().wait()
        x = x_buf[0].astype(jnp.float32)
        xn = _layernorm(x).astype(jnp.bfloat16)
        xn8 = jnp.broadcast_to(xn, (8, D))
        wq_copy().wait()
        q = jnp.dot(xn8, wq_buf[...], preferred_element_type=jnp.float32)
        q_scr[...] = q

        row = lax.broadcasted_iota(jnp.int32, (8, PAIR), 0)
        lane = lax.broadcasted_iota(jnp.int32, (8, PAIR), 1)
        sel = (lane // DH) == row
        scale = DH ** -0.5

        def body(i, carry):
            slot = i % nslots
            off = pl.multiple_of(i * PAIR, 128)
            k_copy(i, slot).wait()
            if compute:
              qp = q_scr[:, pl.ds(off, PAIR)]
              lhs = jnp.where(sel, qp, 0.0).astype(jnp.bfloat16)
              s = jnp.dot(lhs, kbuf[slot], preferred_element_type=jnp.float32) * scale
              m = jnp.max(s, axis=-1, keepdims=True)
              e = jnp.exp(s - m)
              l = jnp.sum(e, axis=-1, keepdims=True)
              eb = e.astype(jnp.bfloat16)
            @pl.when(i + nslots < NPAIR)
            def _():
                k_copy(i + nslots, slot).start()
            v_copy(i, slot).wait()
            if compute:
              o = lax.dot_general(eb, vbuf[slot], (((1,), (1,)), ((), ())),
                                  preferred_element_type=jnp.float32)
              o = o / l
              a_scr[:, pl.ds(off, PAIR)] = jnp.where(sel, o, 0.0)
            @pl.when(i + nslots < NPAIR)
            def _():
                v_copy(i + nslots, slot).start()
            @pl.when(i == NPAIR - nslots)
            def _():
                wo_copy().start()
                w1_copy().start()
                w3_copy().start()
                w2_copy().start()
            return carry

        lax.fori_loop(0, NPAIR, body, 0)

        a = jnp.sum(a_scr[...], axis=0, keepdims=True)
        a8 = jnp.broadcast_to(a.astype(jnp.bfloat16), (8, H * DH))
        wo_copy().wait()
        y = jnp.dot(a8, wo_buf[...], preferred_element_type=jnp.float32)[0:1]
        h = x + y
        hn = jnp.broadcast_to(_layernorm(h).astype(jnp.bfloat16), (8, D))
        w1_copy().wait()
        g = jnp.dot(hn, w1_buf[...], preferred_element_type=jnp.float32)
        w3_copy().wait()
        u = jnp.dot(hn, w3_buf[...], preferred_element_type=jnp.float32)
        act = (g * jax.nn.sigmoid(g) * u).astype(jnp.bfloat16)
        w2_copy().wait()
        z = jnp.dot(act, w2_buf[...], preferred_element_type=jnp.float32)[0:1]
        o_ref[0] = (h + z).astype(o_ref.dtype)

    @jax.jit
    def fn(A_x, A_k_cache, A_v_cache, A_wq, A_wo, B_x, B_w1, B_w3, B_w2):
        kT = jnp.swapaxes(A_k_cache, 2, 3).reshape(H * DH, SK)
        vT = jnp.swapaxes(A_v_cache, 2, 3).reshape(H * DH, SK)
        return pl.pallas_call(
            kernel,
            out_shape=jax.ShapeDtypeStruct((1, 1, D), jnp.bfloat16),
            in_specs=[pl.BlockSpec(memory_space=pl.ANY)] * 8,
            out_specs=pl.BlockSpec(memory_space=pltpu.VMEM),
            scratch_shapes=[
                pltpu.VMEM((1, 1, D), jnp.bfloat16),
                pltpu.VMEM((D, H * DH), jnp.bfloat16),
                pltpu.VMEM((H * DH, D), jnp.bfloat16),
                pltpu.VMEM((D, F), jnp.bfloat16),
                pltpu.VMEM((D, F), jnp.bfloat16),
                pltpu.VMEM((F, D), jnp.bfloat16),
                pltpu.VMEM((nslots, PAIR, W), jnp.bfloat16),
                pltpu.VMEM((nslots, PAIR, W), jnp.bfloat16),
                pltpu.VMEM((8, H * DH), jnp.float32),
                pltpu.VMEM((8, H * DH), jnp.float32),
                pltpu.SemaphoreType.DMA((6,)),
                pltpu.SemaphoreType.DMA((2, nslots)),
            ],
            compiler_params=pltpu.CompilerParams(vmem_limit_bytes=100 * 1024 * 1024),
        )(A_x, kT, vT, A_wq, A_wo, B_w1, B_w3, B_w2)
    return fn


pallas_sequential_preLN__sliding_block_cached__glu_gated_swiglu__decode_kernel = make(nslots=3)
```

```python
import functools
import jax
import jax.numpy as jnp
from jax import lax
from jax.experimental import pallas as pl
from jax.experimental.pallas import tpu as pltpu

D = 640
H = 32
DH = 192
SK = 32768
W = 4096
F = 1536
PAIR = 2 * DH
NPAIR = H // 2
EPS = 1e-5
RT = 16
NRT = PAIR // RT


def _layernorm(x):
    m = jnp.mean(x, axis=-1, keepdims=True)
    c = x - m
    v = jnp.mean(c * c, axis=-1, keepdims=True)
    return c * lax.rsqrt(v + EPS)


def make(kvpat='01011011', wpat='01', L=2, nslots=3, w2chunks=4, cw=1024, split=2):
    kvpat = [int(c) for c in kvpat]
    wpat = [int(c) for c in wpat]
    assert nslots >= L + 1

    def kernel(x_hbm, k_hbm, v_hbm, wq_hbm, wo_hbm, w1_hbm, w3_hbm, w2_hbm, o_ref,
               x_buf, wq_buf, wo_buf, w1_buf, w3_buf, w2_buf, kbuf, vbuf, q_scr, a_scr, p_scr,
               wsem, w2sem, kvsem):
        def full_wait(buf, sem):
            pltpu.make_async_copy(buf, buf, sem).wait()

        nc = W // cw

        def issue_kv(i, g_lo, g_hi):
            slot = i % nslots
            def rbody(r, c_):
                r0 = pl.multiple_of(r * RT, RT)
                n = 0
                for c in range(nc):
                    for t, (src, dst) in enumerate(((k_hbm, kbuf), (v_hbm, vbuf))):
                        pltpu.make_async_copy(
                            src.at[pl.ds(i * PAIR + r0, RT), pl.ds(SK - W + c * cw, cw)],
                            dst.at[slot, pl.ds(r0, RT), pl.ds(c * cw, cw)],
                            kvsem.at[t, slot]).start(priority=kvpat[n % len(kvpat)])
                        n += 1
                return c_
            lax.fori_loop(g_lo, g_hi, rbody, 0)

        def issue_two(srcs, rr, ccw, r_starts, nsteps):
            def rbody(s, c_):
                n = 0
                for rj in range(r_starts[1]):
                    ncol = srcs[0][0].shape[1] // ccw
                    for c in range(ncol):
                        for (src, dst, sem, base) in srcs:
                            r0 = pl.multiple_of(base + (s * r_starts[1] + rj) * rr, RT)
                            pltpu.make_async_copy(
                                src.at[pl.ds(r0, rr), pl.ds(c * ccw, ccw)],
                                dst.at[pl.ds(r0, rr), pl.ds(c * ccw, ccw)],
                                sem).start(priority=wpat[n % len(wpat)])
                            n += 1
                return c_
            lax.fori_loop(r_starts[0], r_starts[0] + nsteps, rbody, 0)

        pltpu.make_async_copy(x_hbm, x_buf, wsem.at[0]).start()
        issue_two([(wq_hbm, wq_buf, wsem.at[1], 0), (wq_hbm, wq_buf, wsem.at[1], D // 2)], RT, 1024, (0, 2), 10)
        issue_kv(0, 0, NRT)

        pltpu.make_async_copy(x_hbm, x_buf, wsem.at[0]).wait()
        x = x_buf[0].astype(jnp.float32)
        xn8 = jnp.broadcast_to(_layernorm(x).astype(jnp.bfloat16), (8, D))
        full_wait(wq_buf, wsem.at[1])
        q_scr[...] = jnp.dot(xn8, wq_buf[...], preferred_element_type=jnp.float32)
        for i in range(1, L):
            issue_kv(i, 0, NRT)

        row = lax.broadcasted_iota(jnp.int32, (8, PAIR), 0)
        lane = lax.broadcasted_iota(jnp.int32, (8, PAIR), 1)
        sel = (lane // DH) == row
        scale = DH ** -0.5

        def qk(i):
            slot = i % nslots
            off = pl.multiple_of(i * PAIR, 128)
            full_wait(kbuf.at[slot], kvsem.at[0, slot])
            qp = q_scr[:, pl.ds(off, PAIR)]
            lhs = jnp.where(sel, qp, 0.0).astype(jnp.bfloat16)
            s = jnp.dot(lhs, kbuf[slot], preferred_element_type=jnp.float32) * scale
            m = jnp.max(s, axis=-1, keepdims=True)
            e = jnp.exp(s - m)
            l = jnp.sum(e, axis=-1, keepdims=True)
            p_scr[...] = (e * (1.0 / l)).astype(jnp.bfloat16)

        def pv(i):
            slot = i % nslots
            off = pl.multiple_of(i * PAIR, 128)
            full_wait(vbuf.at[slot], kvsem.at[1, slot])
            o = lax.dot_general(p_scr[...], vbuf[slot], (((1,), (1,)), ((), ())),
                                preferred_element_type=jnp.float32)
            a_scr[:, pl.ds(off, PAIR)] = jnp.where(sel, o, 0.0)

        def body(i, carry):
            qk(i)
            issue_kv(i + L, 0, NRT // 2)
            pv(i)
            issue_kv(i + L, NRT // 2, NRT)
            return carry
        lax.fori_loop(0, NPAIR - L, body, 0)

        wo_streams = [(wo_hbm, wo_buf, wsem.at[2], 0), (wo_hbm, wo_buf, wsem.at[2], H * DH // 2)]
        w13 = [(w1_hbm, w1_buf, wsem.at[3], 0), (w3_hbm, w3_buf, wsem.at[4], 0)]
        tail_issue = [
            lambda: issue_two(wo_streams, 32, D, (0, 4), 12),
            lambda: issue_two(wo_streams, 32, D, (12, 4), 12),
            lambda: issue_two(w13, RT, 768, (0, 2), 10),
            lambda: issue_two(w13, RT, 768, (10, 2), 10),
        ]
        ti = 0
        per = len(tail_issue) / (2 * L)
        k = 0
        for i in range(NPAIR - L, NPAIR):
            for f in (qk, pv):
                f(i)
                k += 1
                while ti < round(k * per):
                    tail_issue[ti](); ti += 1
        while ti < len(tail_issue):
            tail_issue[ti](); ti += 1

        a = jnp.sum(a_scr[...], axis=0, keepdims=True)
        a8 = jnp.broadcast_to(a.astype(jnp.bfloat16), (8, H * DH))
        full_wait(wo_buf, wsem.at[2])
        y = jnp.dot(a8, wo_buf[...], preferred_element_type=jnp.float32)[0:1]
        h = x + y
        hn = jnp.broadcast_to(_layernorm(h).astype(jnp.bfloat16), (8, D))
        cr = F // w2chunks
        for ch in range(w2chunks):
            n = 0
            for r0 in range(0, cr // 2, 32):
                for half in range(2):
                    rr0 = ch * cr + half * (cr // 2) + r0
                    pltpu.make_async_copy(w2_hbm.at[pl.ds(rr0, 32)], w2_buf.at[pl.ds(rr0, 32)], w2sem.at[ch]).start(priority=wpat[n % len(wpat)])
                    n += 1
        full_wait(w1_buf, wsem.at[3])
        g = jnp.dot(hn, w1_buf[...], preferred_element_type=jnp.float32)
        full_wait(w3_buf, wsem.at[4])
        u = jnp.dot(hn, w3_buf[...], preferred_element_type=jnp.float32)
        act = (g * jax.nn.sigmoid(g) * u).astype(jnp.bfloat16)
        z = h
        for ch in range(w2chunks):
            full_wait(w2_buf.at[pl.ds(ch * cr, cr)], w2sem.at[ch])
            z = z + jnp.dot(act[:, ch * cr:(ch + 1) * cr], w2_buf[pl.ds(ch * cr, cr), :], preferred_element_type=jnp.float32)[0:1]
        o_ref[0] = z.astype(o_ref.dtype)

    @jax.jit
    def fn(A_x, A_k_cache, A_v_cache, A_wq, A_wo, B_x, B_w1, B_w3, B_w2):
        kT = jnp.swapaxes(A_k_cache, 2, 3).reshape(H * DH, SK)
        vT = jnp.swapaxes(A_v_cache, 2, 3).reshape(H * DH, SK)
        return pl.pallas_call(
            kernel,
            out_shape=jax.ShapeDtypeStruct((1, 1, D), jnp.bfloat16),
            in_specs=[pl.BlockSpec(memory_space=pl.ANY)] * 8,
            out_specs=pl.BlockSpec(memory_space=pltpu.VMEM),
            scratch_shapes=[
                pltpu.VMEM((1, 1, D), jnp.bfloat16),
                pltpu.VMEM((D, H * DH), jnp.bfloat16),
                pltpu.VMEM((H * DH, D), jnp.bfloat16),
                pltpu.VMEM((D, F), jnp.bfloat16),
                pltpu.VMEM((D, F), jnp.bfloat16),
                pltpu.VMEM((F, D), jnp.bfloat16),
                pltpu.VMEM((nslots, PAIR, W), jnp.bfloat16),
                pltpu.VMEM((nslots, PAIR, W), jnp.bfloat16),
                pltpu.VMEM((8, H * DH), jnp.float32),
                pltpu.VMEM((8, H * DH), jnp.float32),
                pltpu.VMEM((8, W), jnp.bfloat16),
                pltpu.SemaphoreType.DMA((5,)),
                pltpu.SemaphoreType.DMA((w2chunks,)),
                pltpu.SemaphoreType.DMA((2, nslots)),
            ],
            compiler_params=pltpu.CompilerParams(vmem_limit_bytes=100 * 1024 * 1024),
        )(A_x, kT, vT, A_wq, A_wo, B_w1, B_w3, B_w2)
    return fn


pallas_sequential_preLN__sliding_block_cached__glu_gated_swiglu__decode_kernel = make(kvpat='11111010')
```

```python
import functools
import jax
import jax.numpy as jnp
from jax import lax
from jax.experimental import pallas as pl
from jax.experimental.pallas import tpu as pltpu

D = 640
H = 32
DH = 192
SK = 32768
W = 4096
F = 1536
PAIR = 2 * DH
NPAIR = H // 2
EPS = 1e-5
RT = 8


def _layernorm(x):
    m = jnp.mean(x, axis=-1, keepdims=True)
    c = x - m
    v = jnp.mean(c * c, axis=-1, keepdims=True)
    return c * lax.rsqrt(v + EPS)


def make(kvpat='01011011', kvrows=3, wqpat='01011011', wqparts=8, wopat='01011011', woparts=8, w13pat='01', w13parts=4,
         w2pat='01011011', w2chunks=4, w2parts=2, L=2, nslots=3, tailmode=0):
    P = lambda s: [int(c) for c in s]
    kvpat, wqpat, wopat, w13pat, w2pat = map(P, (kvpat, wqpat, wopat, w13pat, w2pat))
    assert nslots >= L + 1
    CW = W // 2
    NG = PAIR // (RT * kvrows)

    def kernel(x_hbm, k_hbm, v_hbm, wq_hbm, wo_hbm, w1_hbm, w3_hbm, w2_hbm, o_ref,
               x_buf, wq_buf, wo_buf, w1_buf, w3_buf, w2_buf, kbuf, vbuf, q_scr, a_scr, p_scr,
               wsem, w2sem, kvsem):
        def full_wait(buf, sem):
            pltpu.make_async_copy(buf, buf, sem).wait()

        def issue_kv(i, g_lo, g_hi):
            slot = i % nslots
            def rbody(g, c_):
                n = 0
                for c in range(2):
                    for r in range(kvrows):
                        r0 = pl.multiple_of((g * kvrows + r) * RT, RT)
                        for t, (src, dst) in enumerate(((k_hbm, kbuf), (v_hbm, vbuf))):
                            pltpu.make_async_copy(
                                src.at[pl.ds(i * PAIR + r0, RT), pl.ds(SK - W + c * CW, CW)],
                                dst.at[slot, pl.ds(r0, RT), pl.ds(c * CW, CW)],
                                kvsem.at[t, slot]).start(priority=kvpat[n % len(kvpat)])
                            n += 1
                return c_
            lax.fori_loop(g_lo, g_hi, rbody, 0)

        def issue_parts(arrs, rr, ccw, nparts, pat, s_lo, s_hi, unroll=1):
            rows, cols = arrs[0][0].shape
            ncol = cols // ccw
            prow = rows // nparts
            def body(sb, c_):
                n = 0
                for u in range(unroll):
                    for c in range(ncol):
                        for p in range(nparts):
                            r0 = pl.multiple_of(p * prow + (sb * unroll + u) * rr, RT)
                            for (src, dst, sem) in arrs:
                                pltpu.make_async_copy(
                                    src.at[pl.ds(r0, rr), pl.ds(c * ccw, ccw)],
                                    dst.at[pl.ds(r0, rr), pl.ds(c * ccw, ccw)],
                                    sem).start(priority=pat[n % len(pat)])
                                n += 1
                return c_
            lax.fori_loop(s_lo, s_hi, body, 0)

        pltpu.make_async_copy(x_hbm, x_buf, wsem.at[0]).start()
        issue_parts([(wq_hbm, wq_buf, wsem.at[1])], RT, 2048, wqparts, wqpat, 0, D // RT // wqparts)
        issue_kv(0, 0, NG)

        pltpu.make_async_copy(x_hbm, x_buf, wsem.at[0]).wait()
        x = x_buf[0].astype(jnp.float32)
        xn8 = jnp.broadcast_to(_layernorm(x).astype(jnp.bfloat16), (8, D))
        full_wait(wq_buf, wsem.at[1])
        q_scr[...] = jnp.dot(xn8, wq_buf[...], preferred_element_type=jnp.float32)
        for i in range(1, L):
            issue_kv(i, 0, NG)

        row = lax.broadcasted_iota(jnp.int32, (8, PAIR), 0)
        lane = lax.broadcasted_iota(jnp.int32, (8, PAIR), 1)
        sel = (lane // DH) == row
        scale = DH ** -0.5

        def qk(i):
            slot = i % nslots
            off = pl.multiple_of(i * PAIR, 128)
            full_wait(kbuf.at[slot], kvsem.at[0, slot])
            qp = q_scr[:, pl.ds(off, PAIR)]
            lhs = jnp.where(sel, qp, 0.0).astype(jnp.bfloat16)
            s = jnp.dot(lhs, kbuf[slot], preferred_element_type=jnp.float32) * scale
            m = jnp.max(s, axis=-1, keepdims=True)
            e = jnp.exp(s - m)
            l = jnp.sum(e, axis=-1, keepdims=True)
            p_scr[...] = (e * (1.0 / l)).astype(jnp.bfloat16)

        def pv(i):
            slot = i % nslots
            off = pl.multiple_of(i * PAIR, 128)
            full_wait(vbuf.at[slot], kvsem.at[1, slot])
            o = lax.dot_general(p_scr[...], vbuf[slot], (((1,), (1,)), ((), ())),
                                preferred_element_type=jnp.float32)
            a_scr[:, pl.ds(off, PAIR)] = jnp.where(sel, o, 0.0)

        def body(i, carry):
            qk(i)
            issue_kv(i + L, 0, NG // 2)
            pv(i)
            issue_kv(i + L, NG // 2, NG)
            return carry
        lax.fori_loop(0, NPAIR - L, body, 0)

        wo_a = [(wo_hbm, wo_buf, wsem.at[2])]
        w13 = [(w1_hbm, w1_buf, wsem.at[3]), (w3_hbm, w3_buf, wsem.at[4])]
        nwo = H * DH // 16 // woparts
        n13 = D // RT // w13parts
        tail_issue = [
            lambda: issue_parts(wo_a, 16, D, woparts, wopat, 0, nwo // 4, unroll=2),
            lambda: issue_parts(wo_a, 16, D, woparts, wopat, nwo // 4, nwo // 2, unroll=2),
            lambda: issue_parts(w13, RT, F, w13parts, w13pat, 0, n13 // 2),
            lambda: issue_parts(w13, RT, F, w13parts, w13pat, n13 // 2, n13),
        ]
        ti = 0
        per = len(tail_issue) / (2 * L)
        k = 0
        for i in range(NPAIR - L, NPAIR):
            for f in (qk, pv):
                f(i)
                k += 1
                while ti < round(k * per):
                    tail_issue[ti](); ti += 1
        while ti < len(tail_issue):
            tail_issue[ti](); ti += 1

        a = jnp.sum(a_scr[...], axis=0, keepdims=True)
        a8 = jnp.broadcast_to(a.astype(jnp.bfloat16), (8, H * DH))
        full_wait(wo_buf, wsem.at[2])
        y = jnp.dot(a8, wo_buf[...], preferred_element_type=jnp.float32)[0:1]
        h = x + y
        hn = jnp.broadcast_to(_layernorm(h).astype(jnp.bfloat16), (8, D))
        cr = F // w2chunks
        def issue_w2(chunks, pat):
            n = 0
            for ch in chunks:
                pr = cr // w2parts
                for r0 in range(0, pr, 16):
                    for part in range(w2parts):
                        rr0 = ch * cr + part * pr + r0
                        pltpu.make_async_copy(w2_hbm.at[pl.ds(rr0, 16)], w2_buf.at[pl.ds(rr0, 16)], w2sem.at[ch]).start(priority=pat[n % len(pat)])
                        n += 1
        if tailmode == 0:
            issue_w2(range(w2chunks), w2pat)
        elif tailmode == 1:
            issue_w2(range(w2chunks // 2), [1])
        full_wait(w1_buf, wsem.at[3])
        full_wait(w3_buf, wsem.at[4])
        if tailmode == 1:
            issue_w2(range(w2chunks // 2, w2chunks), [0])
        g = jnp.dot(hn, w1_buf[...], preferred_element_type=jnp.float32)
        u = jnp.dot(hn, w3_buf[...], preferred_element_type=jnp.float32)
        act = (g * jax.nn.sigmoid(g) * u).astype(jnp.bfloat16)
        z = h
        for ch in range(w2chunks):
            full_wait(w2_buf.at[pl.ds(ch * cr, cr)], w2sem.at[ch])
            z = z + jnp.dot(act[:, ch * cr:(ch + 1) * cr], w2_buf[pl.ds(ch * cr, cr), :], preferred_element_type=jnp.float32)[0:1]
        o_ref[0] = z.astype(o_ref.dtype)

    @jax.jit
    def fn(A_x, A_k_cache, A_v_cache, A_wq, A_wo, B_x, B_w1, B_w3, B_w2):
        kT = jnp.swapaxes(A_k_cache, 2, 3).reshape(H * DH, SK)
        vT = jnp.swapaxes(A_v_cache, 2, 3).reshape(H * DH, SK)
        return pl.pallas_call(
            kernel,
            out_shape=jax.ShapeDtypeStruct((1, 1, D), jnp.bfloat16),
            in_specs=[pl.BlockSpec(memory_space=pl.ANY)] * 8,
            out_specs=pl.BlockSpec(memory_space=pltpu.VMEM),
            scratch_shapes=[
                pltpu.VMEM((1, 1, D), jnp.bfloat16),
                pltpu.VMEM((D, H * DH), jnp.bfloat16),
                pltpu.VMEM((H * DH, D), jnp.bfloat16),
                pltpu.VMEM((D, F), jnp.bfloat16),
                pltpu.VMEM((D, F), jnp.bfloat16),
                pltpu.VMEM((F, D), jnp.bfloat16),
                pltpu.VMEM((nslots, PAIR, W), jnp.bfloat16),
                pltpu.VMEM((nslots, PAIR, W), jnp.bfloat16),
                pltpu.VMEM((8, H * DH), jnp.float32),
                pltpu.VMEM((8, H * DH), jnp.float32),
                pltpu.VMEM((8, W), jnp.bfloat16),
                pltpu.SemaphoreType.DMA((5,)),
                pltpu.SemaphoreType.DMA((w2chunks,)),
                pltpu.SemaphoreType.DMA((2, nslots)),
            ],
            compiler_params=pltpu.CompilerParams(vmem_limit_bytes=100 * 1024 * 1024),
        )(A_x, kT, vT, A_wq, A_wo, B_w1, B_w3, B_w2)
    return fn


pallas_sequential_preLN__sliding_block_cached__glu_gated_swiglu__decode_kernel = make()
```

```python
import functools
import jax
import jax.numpy as jnp
from jax import lax
from jax.experimental import pallas as pl
from jax.experimental.pallas import tpu as pltpu

D = 640
H = 32
DH = 192
SK = 32768
W = 4096
F = 1536
PAIR = 2 * DH
NPAIR = H // 2
EPS = 1e-5
RT = 8


def _layernorm(x):
    m = jnp.mean(x, axis=-1, keepdims=True)
    c = x - m
    v = jnp.mean(c * c, axis=-1, keepdims=True)
    return c * lax.rsqrt(v + EPS)


def make(kvpat='01011011', kvrows=3, wqpat='01011011', wqparts=8, wopat='01011011', woparts=8, w13pat='01', w13parts=4,
         w2pat='01011011', w2rows=(384,384,384,384), w2parts=2, L=2, nslots=3, tailmode=0, nosemchk=False, nobounds=False, kvorder='cKV'):
    P = lambda s: [int(c) for c in s]
    kvpat, wqpat, wopat, w13pat, w2pat = map(P, (kvpat, wqpat, wopat, w13pat, w2pat))
    assert nslots >= L + 1
    assert sum(w2rows) == F
    w2chunks = len(w2rows)
    w2off = [sum(w2rows[:j]) for j in range(w2chunks)]
    CW = W // 2
    NG = PAIR // (RT * kvrows)

    def kernel(x_hbm, k_hbm, v_hbm, wq_hbm, wo_hbm, w1_hbm, w3_hbm, w2_hbm, o_ref,
               x_buf, wq_buf, wo_buf, w1_buf, w3_buf, w2_buf, kbuf, vbuf, q_scr, a_scr, p_scr,
               wsem, w2sem, kvsem):
        def full_wait(buf, sem):
            pltpu.make_async_copy(buf, buf, sem).wait()

        def issue_kv(i, g_lo, g_hi):
            slot = i % nslots
            def rbody(g, c_):
                if kvorder == 'cKV':
                    items = [(t, r, c) for c in range(2) for r in range(kvrows) for t in range(2)]
                elif kvorder == 'rK':
                    items = [(t, r, c) for c in range(2) for t in range(2) for r in range(kvrows)]
                else:
                    items = [(t, r, c) for t in range(2) for c in range(2) for r in range(kvrows)]
                for n, (t, r, c) in enumerate(items):
                    r0 = pl.multiple_of((g * kvrows + r) * RT, RT)
                    src, dst = ((k_hbm, kbuf), (v_hbm, vbuf))[t]
                    pltpu.make_async_copy(
                        src.at[pl.ds(i * PAIR + r0, RT), pl.ds(SK - W + c * CW, CW)],
                        dst.at[slot, pl.ds(r0, RT), pl.ds(c * CW, CW)],
                        kvsem.at[t, slot]).start(priority=kvpat[n % len(kvpat)])
                return c_
            lax.fori_loop(g_lo, g_hi, rbody, 0)

        def issue_parts(arrs, rr, ccw, nparts, pat, s_lo, s_hi, unroll=1):
            rows, cols = arrs[0][0].shape
            ncol = cols // ccw
            prow = rows // nparts
            def body(sb, c_):
                n = 0
                for u in range(unroll):
                    for c in range(ncol):
                        for p in range(nparts):
                            r0 = pl.multiple_of(p * prow + (sb * unroll + u) * rr, RT)
                            for (src, dst, sem) in arrs:
                                pltpu.make_async_copy(
                                    src.at[pl.ds(r0, rr), pl.ds(c * ccw, ccw)],
                                    dst.at[pl.ds(r0, rr), pl.ds(c * ccw, ccw)],
                                    sem).start(priority=pat[n % len(pat)])
                                n += 1
                return c_
            lax.fori_loop(s_lo, s_hi, body, 0)

        pltpu.make_async_copy(x_hbm, x_buf, wsem.at[0]).start()
        issue_parts([(wq_hbm, wq_buf, wsem.at[1])], RT, 2048, wqparts, wqpat, 0, D // RT // wqparts)
        issue_kv(0, 0, NG)

        pltpu.make_async_copy(x_hbm, x_buf, wsem.at[0]).wait()
        x = x_buf[0].astype(jnp.float32)
        xn8 = jnp.broadcast_to(_layernorm(x).astype(jnp.bfloat16), (8, D))
        full_wait(wq_buf, wsem.at[1])
        q_scr[...] = jnp.dot(xn8, wq_buf[...], preferred_element_type=jnp.float32)
        for i in range(1, L):
            issue_kv(i, 0, NG)

        row = lax.broadcasted_iota(jnp.int32, (8, PAIR), 0)
        lane = lax.broadcasted_iota(jnp.int32, (8, PAIR), 1)
        sel = (lane // DH) == row
        scale = DH ** -0.5

        def qk(i):
            slot = i % nslots
            off = pl.multiple_of(i * PAIR, 128)
            full_wait(kbuf.at[slot], kvsem.at[0, slot])
            qp = q_scr[:, pl.ds(off, PAIR)]
            lhs = jnp.where(sel, qp, 0.0).astype(jnp.bfloat16)
            s = jnp.dot(lhs, kbuf[slot], preferred_element_type=jnp.float32) * scale
            m = jnp.max(s, axis=-1, keepdims=True)
            e = jnp.exp(s - m)
            l = jnp.sum(e, axis=-1, keepdims=True)
            p_scr[...] = (e * (1.0 / l)).astype(jnp.bfloat16)

        def pv(i):
            slot = i % nslots
            off = pl.multiple_of(i * PAIR, 128)
            full_wait(vbuf.at[slot], kvsem.at[1, slot])
            o = lax.dot_general(p_scr[...], vbuf[slot], (((1,), (1,)), ((), ())),
                                preferred_element_type=jnp.float32)
            a_scr[:, pl.ds(off, PAIR)] = jnp.where(sel, o, 0.0)

        def body(i, carry):
            qk(i)
            issue_kv(i + L, 0, NG // 2)
            pv(i)
            issue_kv(i + L, NG // 2, NG)
            return carry
        lax.fori_loop(0, NPAIR - L, body, 0)

        wo_a = [(wo_hbm, wo_buf, wsem.at[2])]
        w13 = [(w1_hbm, w1_buf, wsem.at[3]), (w3_hbm, w3_buf, wsem.at[4])]
        nwo = H * DH // 16 // woparts
        n13 = D // RT // w13parts
        tail_issue = [
            lambda: issue_parts(wo_a, 16, D, woparts, wopat, 0, nwo // 4, unroll=2),
            lambda: issue_parts(wo_a, 16, D, woparts, wopat, nwo // 4, nwo // 2, unroll=2),
            lambda: issue_parts(w13, RT, F, w13parts, w13pat, 0, n13 // 2),
            lambda: issue_parts(w13, RT, F, w13parts, w13pat, n13 // 2, n13),
        ]
        ti = 0
        per = len(tail_issue) / (2 * L)
        k = 0
        for i in range(NPAIR - L, NPAIR):
            for f in (qk, pv):
                f(i)
                k += 1
                while ti < round(k * per):
                    tail_issue[ti](); ti += 1
        while ti < len(tail_issue):
            tail_issue[ti](); ti += 1

        a = jnp.sum(a_scr[...], axis=0, keepdims=True)
        a8 = jnp.broadcast_to(a.astype(jnp.bfloat16), (8, H * DH))
        full_wait(wo_buf, wsem.at[2])
        y = jnp.dot(a8, wo_buf[...], preferred_element_type=jnp.float32)[0:1]
        h = x + y
        hn = jnp.broadcast_to(_layernorm(h).astype(jnp.bfloat16), (8, D))
        def issue_w2(chunks, pat):
            n = 0
            for ch in chunks:
                pr = w2rows[ch] // w2parts
                for r0 in range(0, pr, 16):
                    for part in range(w2parts):
                        rr0 = w2off[ch] + part * pr + r0
                        pltpu.make_async_copy(w2_hbm.at[pl.ds(rr0, 16)], w2_buf.at[pl.ds(rr0, 16)], w2sem.at[ch]).start(priority=pat[n % len(pat)])
                        n += 1
        if tailmode == 0:
            issue_w2(range(w2chunks), w2pat)
        elif tailmode == 1:
            issue_w2(range(w2chunks // 2), [1])
        full_wait(w1_buf, wsem.at[3])
        full_wait(w3_buf, wsem.at[4])
        if tailmode == 1:
            issue_w2(range(w2chunks // 2, w2chunks), [0])
        g = jnp.dot(hn, w1_buf[...], preferred_element_type=jnp.float32)
        u = jnp.dot(hn, w3_buf[...], preferred_element_type=jnp.float32)
        act = (g * jax.nn.sigmoid(g) * u).astype(jnp.bfloat16)
        z = h
        for ch in range(w2chunks):
            lo, cr = w2off[ch], w2rows[ch]
            full_wait(w2_buf.at[pl.ds(lo, cr)], w2sem.at[ch])
            z = z + jnp.dot(act[:, lo:lo + cr], w2_buf[pl.ds(lo, cr), :], preferred_element_type=jnp.float32)[0:1]
        o_ref[0] = z.astype(o_ref.dtype)

    @jax.jit
    def fn(A_x, A_k_cache, A_v_cache, A_wq, A_wo, B_x, B_w1, B_w3, B_w2):
        kT = jnp.swapaxes(A_k_cache, 2, 3).reshape(H * DH, SK)
        vT = jnp.swapaxes(A_v_cache, 2, 3).reshape(H * DH, SK)
        return pl.pallas_call(
            kernel,
            out_shape=jax.ShapeDtypeStruct((1, 1, D), jnp.bfloat16),
            in_specs=[pl.BlockSpec(memory_space=pl.ANY)] * 8,
            out_specs=pl.BlockSpec(memory_space=pltpu.VMEM),
            scratch_shapes=[
                pltpu.VMEM((1, 1, D), jnp.bfloat16),
                pltpu.VMEM((D, H * DH), jnp.bfloat16),
                pltpu.VMEM((H * DH, D), jnp.bfloat16),
                pltpu.VMEM((D, F), jnp.bfloat16),
                pltpu.VMEM((D, F), jnp.bfloat16),
                pltpu.VMEM((F, D), jnp.bfloat16),
                pltpu.VMEM((nslots, PAIR, W), jnp.bfloat16),
                pltpu.VMEM((nslots, PAIR, W), jnp.bfloat16),
                pltpu.VMEM((8, H * DH), jnp.float32),
                pltpu.VMEM((8, H * DH), jnp.float32),
                pltpu.VMEM((8, W), jnp.bfloat16),
                pltpu.SemaphoreType.DMA((5,)),
                pltpu.SemaphoreType.DMA((w2chunks,)),
                pltpu.SemaphoreType.DMA((2, nslots)),
            ],
            compiler_params=pltpu.CompilerParams(vmem_limit_bytes=100 * 1024 * 1024, disable_semaphore_checks=nosemchk, disable_bounds_checks=nobounds),
        )(A_x, kT, vT, A_wq, A_wo, B_w1, B_w3, B_w2)
    return fn


pallas_sequential_preLN__sliding_block_cached__glu_gated_swiglu__decode_kernel = make(
    nosemchk=True, w2rows=(768, 512, 256), kvrows=12, kvpat='01', kvorder='KKVV', w2pat='01', wqpat='0111', wopat='0111')
```

```python
import jax
import jax.numpy as jnp
from jax import lax
import jax.experimental.pallas as pl
import jax.experimental.pallas.tpu as pltpu

D = 640
H = 32
DH = 192
SK = 32768
W = min(4096, max(256, SK // 4))
F = 1536
EPS = 1e-5

PAIR = 2 * DH
NPAIR = H // 2
TILE_ROWS = 8

NSLOTS = 3
AHEAD = 2
KV_COLS = 2048
KV_GROUP = 12
KV_GROUPS = PAIR // (TILE_ROWS * KV_GROUP)

WQ_PARTS = 8
WO_PARTS = 8
W13_PARTS = 4
W2_CHUNKS = (768, 512, 256)

ALTERNATE = (0, 1)
ONE_IN_FOUR = (0, 1, 1, 1)

_VMEM_LIMIT = 64 * 1024 * 1024


def _layernorm(x):
    mean = jnp.mean(x, axis=-1, keepdims=True)
    c = x - mean
    var = jnp.mean(c * c, axis=-1, keepdims=True)
    return c * lax.rsqrt(var + EPS)


def _wait_all(buf, sem):
    pltpu.make_async_copy(buf, buf, sem).wait()


def _rows8(v):
    return jnp.broadcast_to(v.astype(jnp.bfloat16), (8, v.shape[-1]))


def _kernel(x_hbm, k_hbm, v_hbm, wq_hbm, wo_hbm, w1_hbm, w3_hbm, w2_hbm, o_ref,
            x_buf, wq_buf, wo_buf, w1_buf, w3_buf, w2_buf, k_buf, v_buf,
            q_scr, attn_scr, p_scr, w_sem, w2_sem, kv_sem):

    def start_kv(pair, g_lo, g_hi):
        slot = pair % NSLOTS

        def group(g, carry):
            n = 0
            for t, (src, dst) in enumerate(((k_hbm, k_buf), (v_hbm, v_buf))):
                for c in range(W // KV_COLS):
                    for r in range(KV_GROUP):
                        r0 = pl.multiple_of((g * KV_GROUP + r) * TILE_ROWS, TILE_ROWS)
                        pltpu.make_async_copy(
                            src.at[pl.ds(pair * PAIR + r0, TILE_ROWS),
                                   pl.ds(SK - W + c * KV_COLS, KV_COLS)],
                            dst.at[slot, pl.ds(r0, TILE_ROWS), pl.ds(c * KV_COLS, KV_COLS)],
                            kv_sem.at[t, slot],
                        ).start(priority=ALTERNATE[n % 2])
                        n += 1
            return carry

        lax.fori_loop(g_lo, g_hi, group, 0)

    def start_weights(arrays, rows, cols, parts, prio, s_lo, s_hi, unroll=1):
        n_rows, n_cols = arrays[0][0].shape
        part_rows = n_rows // parts

        def step(s, carry):
            n = 0
            for u in range(unroll):
                for c in range(n_cols // cols):
                    for p in range(parts):
                        r0 = pl.multiple_of(p * part_rows + (s * unroll + u) * rows, TILE_ROWS)
                        for src, dst, sem in arrays:
                            pltpu.make_async_copy(
                                src.at[pl.ds(r0, rows), pl.ds(c * cols, cols)],
                                dst.at[pl.ds(r0, rows), pl.ds(c * cols, cols)],
                                sem,
                            ).start(priority=prio[n % len(prio)])
                            n += 1
            return carry

        lax.fori_loop(s_lo, s_hi, step, 0)

    x_copy = pltpu.make_async_copy(x_hbm, x_buf, w_sem.at[0])
    x_copy.start()
    start_weights([(wq_hbm, wq_buf, w_sem.at[1])], TILE_ROWS, 2048, WQ_PARTS, ONE_IN_FOUR,
                  0, D // TILE_ROWS // WQ_PARTS)
    start_kv(0, 0, KV_GROUPS)

    x_copy.wait()
    x = x_buf[0].astype(jnp.float32)
    _wait_all(wq_buf, w_sem.at[1])
    q_scr[...] = jnp.dot(_rows8(_layernorm(x)), wq_buf[...],
                         preferred_element_type=jnp.float32)
    for pair in range(1, AHEAD):
        start_kv(pair, 0, KV_GROUPS)

    own = (lax.broadcasted_iota(jnp.int32, (8, PAIR), 1) // DH
           == lax.broadcasted_iota(jnp.int32, (8, PAIR), 0))

    def scores_softmax(pair):
        slot = pair % NSLOTS
        cols = pl.ds(pl.multiple_of(pair * PAIR, 128), PAIR)
        _wait_all(k_buf.at[slot], kv_sem.at[0, slot])
        q = jnp.where(own, q_scr[:, cols], 0.0).astype(jnp.bfloat16)
        s = jnp.dot(q, k_buf[slot], preferred_element_type=jnp.float32) * (DH ** -0.5)
        e = jnp.exp(s - jnp.max(s, axis=-1, keepdims=True))
        p_scr[...] = (e * (1.0 / jnp.sum(e, axis=-1, keepdims=True))).astype(jnp.bfloat16)

    def weighted_values(pair):
        slot = pair % NSLOTS
        cols = pl.ds(pl.multiple_of(pair * PAIR, 128), PAIR)
        _wait_all(v_buf.at[slot], kv_sem.at[1, slot])
        o = lax.dot_general(p_scr[...], v_buf[slot], (((1,), (1,)), ((), ())),
                            preferred_element_type=jnp.float32)
        attn_scr[:, cols] = jnp.where(own, o, 0.0)

    def pair_step(pair, carry):
        scores_softmax(pair)
        start_kv(pair + AHEAD, 0, KV_GROUPS // 2)
        weighted_values(pair)
        start_kv(pair + AHEAD, KV_GROUPS // 2, KV_GROUPS)
        return carry

    lax.fori_loop(0, NPAIR - AHEAD, pair_step, 0)

    wo = [(wo_hbm, wo_buf, w_sem.at[2])]
    w13 = [(w1_hbm, w1_buf, w_sem.at[3]), (w3_hbm, w3_buf, w_sem.at[4])]
    wo_steps = H * DH // (2 * TILE_ROWS) // WO_PARTS // 2
    w13_steps = D // TILE_ROWS // W13_PARTS
    scores_softmax(NPAIR - 2)
    start_weights(wo, 2 * TILE_ROWS, D, WO_PARTS, ONE_IN_FOUR, 0, wo_steps // 2, unroll=2)
    weighted_values(NPAIR - 2)
    start_weights(wo, 2 * TILE_ROWS, D, WO_PARTS, ONE_IN_FOUR, wo_steps // 2, wo_steps, unroll=2)
    scores_softmax(NPAIR - 1)
    start_weights(w13, TILE_ROWS, F, W13_PARTS, ALTERNATE, 0, w13_steps // 2)
    weighted_values(NPAIR - 1)
    start_weights(w13, TILE_ROWS, F, W13_PARTS, ALTERNATE, w13_steps // 2, w13_steps)

    attn = jnp.sum(attn_scr[...], axis=0, keepdims=True)
    _wait_all(wo_buf, w_sem.at[2])
    h = x + jnp.dot(_rows8(attn), wo_buf[...], preferred_element_type=jnp.float32)[0:1]
    hn = _rows8(_layernorm(h))

    n = 0
    lo = 0
    for ch, rows in enumerate(W2_CHUNKS):
        for r in range(0, rows // 2, 2 * TILE_ROWS):
            for half in range(2):
                piece = pl.ds(lo + half * (rows // 2) + r, 2 * TILE_ROWS)
                pltpu.make_async_copy(w2_hbm.at[piece], w2_buf.at[piece],
                                      w2_sem.at[ch]).start(priority=ALTERNATE[n % 2])
                n += 1
        lo += rows

    _wait_all(w1_buf, w_sem.at[3])
    _wait_all(w3_buf, w_sem.at[4])
    gate = jnp.dot(hn, w1_buf[...], preferred_element_type=jnp.float32)
    up = jnp.dot(hn, w3_buf[...], preferred_element_type=jnp.float32)
    act = (gate * jax.nn.sigmoid(gate) * up).astype(jnp.bfloat16)

    out = h
    lo = 0
    for ch, rows in enumerate(W2_CHUNKS):
        _wait_all(w2_buf.at[pl.ds(lo, rows)], w2_sem.at[ch])
        out = out + jnp.dot(act[:, lo:lo + rows], w2_buf[pl.ds(lo, rows), :],
                            preferred_element_type=jnp.float32)[0:1]
        lo += rows
    o_ref[0] = out.astype(o_ref.dtype)


@jax.jit
def pallas_sequential_preLN__sliding_block_cached__glu_gated_swiglu__decode_kernel(
    A_x: jax.Array,
    A_k_cache: jax.Array,
    A_v_cache: jax.Array,
    A_wq: jax.Array,
    A_wo: jax.Array,
    B_x: jax.Array,
    B_w1: jax.Array,
    B_w3: jax.Array,
    B_w2: jax.Array,
):
    del B_x
    k_t = jnp.swapaxes(A_k_cache, 2, 3).reshape(H * DH, SK)
    v_t = jnp.swapaxes(A_v_cache, 2, 3).reshape(H * DH, SK)

    params = dict(vmem_limit_bytes=_VMEM_LIMIT)
    if hasattr(pltpu.CompilerParams, "disable_semaphore_checks"):
        params["disable_semaphore_checks"] = True

    return pl.pallas_call(
        _kernel,
        out_shape=jax.ShapeDtypeStruct((1, 1, D), A_x.dtype),
        in_specs=[pl.BlockSpec(memory_space=pl.ANY)] * 8,
        out_specs=pl.BlockSpec(memory_space=pltpu.VMEM),
        scratch_shapes=[
            pltpu.VMEM((1, 1, D), jnp.bfloat16),
            pltpu.VMEM((D, H * DH), jnp.bfloat16),
            pltpu.VMEM((H * DH, D), jnp.bfloat16),
            pltpu.VMEM((D, F), jnp.bfloat16),
            pltpu.VMEM((D, F), jnp.bfloat16),
            pltpu.VMEM((F, D), jnp.bfloat16),
            pltpu.VMEM((NSLOTS, PAIR, W), jnp.bfloat16),
            pltpu.VMEM((NSLOTS, PAIR, W), jnp.bfloat16),
            pltpu.VMEM((8, H * DH), jnp.float32),
            pltpu.VMEM((8, H * DH), jnp.float32),
            pltpu.VMEM((8, W), jnp.bfloat16),
            pltpu.SemaphoreType.DMA((5,)),
            pltpu.SemaphoreType.DMA((len(W2_CHUNKS),)),
            pltpu.SemaphoreType.DMA((2, NSLOTS)),
        ],
        compiler_params=pltpu.CompilerParams(**params),
    )(A_x, k_t, v_t, A_wq, A_wo, B_w1, B_w3, B_w2)
```

```python
import jax
import jax.numpy as jnp
from jax import lax
import jax.experimental.pallas as pl
import jax.experimental.pallas.tpu as pltpu

D = 640
H = 32
DH = 192
SK = 32768
W = min(4096, max(256, SK // 4))
F = 1536
EPS = 1e-5

PAIR = 2 * DH
NPAIR = H // 2
TILE_ROWS = 8

NSLOTS = 3
AHEAD = 2
KV_COLS = 2048
KV_GROUP = 12
KV_GROUPS = PAIR // (TILE_ROWS * KV_GROUP)

WQ_PARTS = 8
WO_PARTS = 8
W13_PARTS = 4
W2_CHUNKS = (768, 512, 256)

ALTERNATE = (0, 1)
ONE_IN_FOUR = (0, 1, 1, 1)

_VMEM_LIMIT = 64 * 1024 * 1024


def _layernorm(x):
    mean = jnp.mean(x, axis=-1, keepdims=True)
    c = x - mean
    var = jnp.mean(c * c, axis=-1, keepdims=True)
    return c * lax.rsqrt(var + EPS)


def _wait_all(buf, sem):
    pltpu.make_async_copy(buf, buf, sem).wait()


def _rows8(v):
    return jnp.broadcast_to(v.astype(jnp.bfloat16), (8, v.shape[-1]))


def _kernel(x_hbm, k_hbm, v_hbm, wq_hbm, wo_hbm, w1_hbm, w3_hbm, w2_hbm, o_ref,
            x_buf, wq_buf, wo_buf, w1_buf, w3_buf, w2_buf, k_buf, v_buf,
            q_scr, attn_scr, p_scr, w_sem, w2_sem, kv_sem):

    def start_kv(pair, g_lo, g_hi):
        slot = pair % NSLOTS

        def group(g, carry):
            n = 0
            for t, (src, dst) in enumerate(((k_hbm, k_buf), (v_hbm, v_buf))):
                for c in range(W // KV_COLS):
                    for r in range(KV_GROUP):
                        r0 = pl.multiple_of((g * KV_GROUP + r) * TILE_ROWS, TILE_ROWS)
                        pltpu.make_async_copy(
                            src.at[pl.ds(pair * PAIR + r0, TILE_ROWS),
                                   pl.ds(SK - W + c * KV_COLS, KV_COLS)],
                            dst.at[slot, pl.ds(r0, TILE_ROWS), pl.ds(c * KV_COLS, KV_COLS)],
                            kv_sem.at[t, slot],
                        ).start(priority=ALTERNATE[n % 2])
                        n += 1
            return carry

        lax.fori_loop(g_lo, g_hi, group, 0)

    def start_weights(arrays, rows, cols, parts, prio, s_lo, s_hi, unroll=1):
        n_rows, n_cols = arrays[0][0].shape
        part_rows = n_rows // parts

        def step(s, carry):
            n = 0
            for u in range(unroll):
                for c in range(n_cols // cols):
                    for p in range(parts):
                        r0 = pl.multiple_of(p * part_rows + (s * unroll + u) * rows, TILE_ROWS)
                        for src, dst, sem in arrays:
                            pltpu.make_async_copy(
                                src.at[pl.ds(r0, rows), pl.ds(c * cols, cols)],
                                dst.at[pl.ds(r0, rows), pl.ds(c * cols, cols)],
                                sem,
                            ).start(priority=prio[n % len(prio)])
                            n += 1
            return carry

        lax.fori_loop(s_lo, s_hi, step, 0)

    x_copy = pltpu.make_async_copy(x_hbm, x_buf, w_sem.at[0])
    x_copy.start()
    start_weights([(wq_hbm, wq_buf, w_sem.at[1])], TILE_ROWS, 2048, WQ_PARTS, ONE_IN_FOUR,
                  0, D // TILE_ROWS // WQ_PARTS)
    start_kv(0, 0, KV_GROUPS)

    x_copy.wait()
    x = x_buf[0].astype(jnp.float32)
    _wait_all(wq_buf, w_sem.at[1])
    q_scr[...] = jnp.dot(_rows8(_layernorm(x)), wq_buf[...],
                         preferred_element_type=jnp.float32)
    for pair in range(1, AHEAD):
        start_kv(pair, 0, KV_GROUPS)

    own = (lax.broadcasted_iota(jnp.int32, (8, PAIR), 1) // DH
           == lax.broadcasted_iota(jnp.int32, (8, PAIR), 0))

    def scores_softmax(pair):
        slot = pair % NSLOTS
        cols = pl.ds(pl.multiple_of(pair * PAIR, 128), PAIR)
        _wait_all(k_buf.at[slot], kv_sem.at[0, slot])
        q = q_scr[:, cols].astype(jnp.bfloat16)

        def part(lo, hi):
            return jnp.dot(q[:, lo:hi], k_buf[slot, lo:hi, :], preferred_element_type=jnp.float32)

        s_first = part(0, 128) + part(128, DH)
        s_second = part(DH, 256) + part(256, PAIR)
        s = jnp.where(lax.broadcasted_iota(jnp.int32, (8, W), 0) == 0, s_first, s_second) * (DH ** -0.5)
        e = jnp.exp(s - jnp.max(s, axis=-1, keepdims=True))
        p_scr[...] = (e * (1.0 / jnp.sum(e, axis=-1, keepdims=True))).astype(jnp.bfloat16)

    def weighted_values(pair):
        slot = pair % NSLOTS
        cols = pl.ds(pl.multiple_of(pair * PAIR, 128), PAIR)
        _wait_all(v_buf.at[slot], kv_sem.at[1, slot])
        o = lax.dot_general(p_scr[...], v_buf[slot], (((1,), (1,)), ((), ())),
                            preferred_element_type=jnp.float32)
        attn_scr[:, cols] = jnp.where(own, o, 0.0)

    def pair_step(pair, carry):
        scores_softmax(pair)
        start_kv(pair + AHEAD, 0, KV_GROUPS // 2)
        weighted_values(pair)
        start_kv(pair + AHEAD, KV_GROUPS // 2, KV_GROUPS)
        return carry

    lax.fori_loop(0, NPAIR - AHEAD, pair_step, 0)

    wo = [(wo_hbm, wo_buf, w_sem.at[2])]
    w13 = [(w1_hbm, w1_buf, w_sem.at[3]), (w3_hbm, w3_buf, w_sem.at[4])]
    wo_steps = H * DH // (2 * TILE_ROWS) // WO_PARTS // 2
    w13_steps = D // TILE_ROWS // W13_PARTS
    scores_softmax(NPAIR - 2)
    start_weights(wo, 2 * TILE_ROWS, D, WO_PARTS, ONE_IN_FOUR, 0, wo_steps // 2, unroll=2)
    weighted_values(NPAIR - 2)
    start_weights(wo, 2 * TILE_ROWS, D, WO_PARTS, ONE_IN_FOUR, wo_steps // 2, wo_steps, unroll=2)
    scores_softmax(NPAIR - 1)
    start_weights(w13, TILE_ROWS, F, W13_PARTS, ALTERNATE, 0, w13_steps // 2)
    weighted_values(NPAIR - 1)
    start_weights(w13, TILE_ROWS, F, W13_PARTS, ALTERNATE, w13_steps // 2, w13_steps)

    attn = jnp.sum(attn_scr[...], axis=0, keepdims=True)
    _wait_all(wo_buf, w_sem.at[2])
    h = x + jnp.dot(_rows8(attn), wo_buf[...], preferred_element_type=jnp.float32)[0:1]
    hn = _rows8(_layernorm(h))

    n = 0
    lo = 0
    for ch, rows in enumerate(W2_CHUNKS):
        for r in range(0, rows // 2, 2 * TILE_ROWS):
            for half in range(2):
                piece = pl.ds(lo + half * (rows // 2) + r, 2 * TILE_ROWS)
                pltpu.make_async_copy(w2_hbm.at[piece], w2_buf.at[piece],
                                      w2_sem.at[ch]).start(priority=ALTERNATE[n % 2])
                n += 1
        lo += rows

    _wait_all(w1_buf, w_sem.at[3])
    _wait_all(w3_buf, w_sem.at[4])
    gate = jnp.dot(hn, w1_buf[...], preferred_element_type=jnp.float32)
    up = jnp.dot(hn, w3_buf[...], preferred_element_type=jnp.float32)
    act = (gate * jax.nn.sigmoid(gate) * up).astype(jnp.bfloat16)

    out = h
    lo = 0
    for ch, rows in enumerate(W2_CHUNKS):
        _wait_all(w2_buf.at[pl.ds(lo, rows)], w2_sem.at[ch])
        out = out + jnp.dot(act[:, lo:lo + rows], w2_buf[pl.ds(lo, rows), :],
                            preferred_element_type=jnp.float32)[0:1]
        lo += rows
    o_ref[0] = out.astype(o_ref.dtype)


@jax.jit
def pallas_sequential_preLN__sliding_block_cached__glu_gated_swiglu__decode_kernel(
    A_x: jax.Array,
    A_k_cache: jax.Array,
    A_v_cache: jax.Array,
    A_wq: jax.Array,
    A_wo: jax.Array,
    B_x: jax.Array,
    B_w1: jax.Array,
    B_w3: jax.Array,
    B_w2: jax.Array,
):
    del B_x
    k_t = jnp.swapaxes(A_k_cache, 2, 3).reshape(H * DH, SK)
    v_t = jnp.swapaxes(A_v_cache, 2, 3).reshape(H * DH, SK)

    params = dict(vmem_limit_bytes=_VMEM_LIMIT)
    if hasattr(pltpu.CompilerParams, "disable_semaphore_checks"):
        params["disable_semaphore_checks"] = True

    return pl.pallas_call(
        _kernel,
        out_shape=jax.ShapeDtypeStruct((1, 1, D), A_x.dtype),
        in_specs=[pl.BlockSpec(memory_space=pl.ANY)] * 8,
        out_specs=pl.BlockSpec(memory_space=pltpu.VMEM),
        scratch_shapes=[
            pltpu.VMEM((1, 1, D), jnp.bfloat16),
            pltpu.VMEM((D, H * DH), jnp.bfloat16),
            pltpu.VMEM((H * DH, D), jnp.bfloat16),
            pltpu.VMEM((D, F), jnp.bfloat16),
            pltpu.VMEM((D, F), jnp.bfloat16),
            pltpu.VMEM((F, D), jnp.bfloat16),
            pltpu.VMEM((NSLOTS, PAIR, W), jnp.bfloat16),
            pltpu.VMEM((NSLOTS, PAIR, W), jnp.bfloat16),
            pltpu.VMEM((8, H * DH), jnp.float32),
            pltpu.VMEM((8, H * DH), jnp.float32),
            pltpu.VMEM((8, W), jnp.bfloat16),
            pltpu.SemaphoreType.DMA((5,)),
            pltpu.SemaphoreType.DMA((len(W2_CHUNKS),)),
            pltpu.SemaphoreType.DMA((2, NSLOTS)),
        ],
        compiler_params=pltpu.CompilerParams(**params),
    )(A_x, k_t, v_t, A_wq, A_wo, B_w1, B_w3, B_w2)
```
